```python
import jax
import jax.numpy as jnp

def _softmax(x, axis=-1):
    return jax.nn.softmax(x, axis=axis)
def _gelu(x):
    return jax.nn.gelu(x, approximate=True)
def _silu(x):
    return jax.nn.silu(x)
def _sigmoid(x):
    return jax.nn.sigmoid(x)
def _layernorm(x, axis=-1, eps=1e-5):
    m = jnp.mean(x, axis=axis, keepdims=True)
    v = jnp.var(x, axis=axis, keepdims=True)
    return (x - m) / jnp.sqrt(v + eps)
def _scatter_add(tgt, idx, src, axis=0):
    return tgt.at[idx].add(src)
def _segment_sum(src, seg, n):
    return jax.ops.segment_sum(src, seg, n)
class _Rng:
    def __init__(self, key):
        self._k = key
    def _next(self):
        self._k, sub = jax.random.split(self._k)
        return sub
    def normal(self, shape):
        return jax.random.normal(self._next(), shape, dtype=jnp.bfloat16)
    def randint(self, lo, hi, shape):
        return jax.random.randint(self._next(), shape, lo, hi, dtype=jnp.int32)
    def uniform(self, shape, lo=0.0, hi=1.0):
        return jax.random.uniform(self._next(), shape, jnp.bfloat16, lo, hi)
    def permutation(self, n):
        return jax.random.permutation(self._next(), n)


kernel_name = 'interleave_layers__sliding_block_cached__moe_arch_mod__decode'

def setup_inputs():
    _rng = _Rng(jax.random.key(int.from_bytes(__import__("os").urandom(4), "little")))
    _w = (lambda a: (lambda t: t.astype(jnp.bfloat16) if jnp.issubdtype(t.dtype, jnp.floating) else t)(jnp.asarray(a)))
    def _A_setup():
        B, Sq, D = 4, 1, 640
        Hq, Hkv, Sk, Dh = 32, 32, 4096, 192
        assert Hq % Hkv == 0, (Hq, Hkv)
        return {
            "x": _w((lambda *s: _rng.normal(s) * 0.05)(B, Sq, D)),
            "k_cache": _w((lambda *s: _rng.normal(s) * 0.05)(B, Hkv, Sk, Dh)),
            "v_cache": _w((lambda *s: _rng.normal(s) * 0.05)(B, Hkv, Sk, Dh)),
            "wq": _w((lambda *s: _rng.normal(s) * 0.05)(D, Hq * Dh) * (D ** -0.5)),
            "wo": _w((lambda *s: _rng.normal(s) * 0.05)(Hq * Dh, D) * ((Hq * Dh) ** -0.5)),
        }
    _A_in = _A_setup()

    def _B_setup():
        B, S, D, F, C = 4, 1, 640, 1536, 1
        return {
            "x": _w((lambda *s: _rng.normal(s) * 0.05)(B, S, D)),
            "w_r": _w((lambda *s: _rng.normal(s) * 0.05)(D)),
            "w_gate": _w((lambda *s: _rng.normal(s) * 0.05)(D, F)),
            "w_up": _w((lambda *s: _rng.normal(s) * 0.05)(D, F)),
            "w_down": _w((lambda *s: _rng.normal(s) * 0.05)(F, D)),
        }
    _B_in = _B_setup()

    return {
        "A_x": _A_in["x"],
        "A_k_cache": _A_in["k_cache"],
        "A_v_cache": _A_in["v_cache"],
        "A_wq": _A_in["wq"],
        "A_wo": _A_in["wo"],
        "B_x": _B_in["x"],
        "B_w_r": _B_in["w_r"],
        "B_w_gate": _B_in["w_gate"],
        "B_w_up": _B_in["w_up"],
        "B_w_down": _B_in["w_down"],
    }

def reference(A_x, A_k_cache, A_v_cache, A_wq, A_wo, B_x, B_w_r, B_w_gate, B_w_up, B_w_down):
    def _A_ref(x, k_cache, v_cache, wq, wo):
        B, Sq, D = x.shape
        Hq, Dh = 32, 192
        Hkv, Sk = k_cache.shape[1], k_cache.shape[2]
        W = min(4096, max(256, Sk // 4))
        rep = Hq // Hkv
        q = (lambda x, *d: x.transpose(*d))((x @ wq).reshape(B, Sq, Hq, Dh), 0, 2, 1, 3)
        k = jnp.repeat(k_cache[:, :, Sk - W:, :], rep, axis=1)
        v = jnp.repeat(v_cache[:, :, Sk - W:, :], rep, axis=1)
        scores = jnp.einsum("bhqd,bhkd->bhqk", q, k) * (Dh ** -0.5)
        p = _softmax(scores, axis=-1)
        o = jnp.einsum("bhqk,bhkd->bhqd", p, v)
        return (lambda x, *d: x.transpose(*d))(o, 0, 2, 1, 3).reshape(B, Sq, Hq * Dh) @ wo

    def _B_ref(x, w_r, w_gate, w_up, w_down):
        B, S, D = x.shape
        C = 1
        r = x @ w_r
        idx = jnp.argsort(-r, axis=-1)[:, :C]
        idx_e = jnp.repeat(idx.reshape(B, C, 1), D, axis=2)
        x_sel = jnp.take_along_axis(x, idx_e, axis=1)
        g = _silu(x_sel @ w_gate)
        u = x_sel @ w_up
        y = (g * u) @ w_down
        r_sel = _sigmoid(jnp.take_along_axis(r, idx, axis=1))
        y = y * r_sel.reshape(B, C, 1)
        b_off = (jnp.arange(B) * S).reshape(B, 1)
        flat_idx = (idx + b_off).reshape(B * C)
        zero = (x * 0.0).reshape(B * S, D)
        upd = _scatter_add(zero, flat_idx, y.reshape(B * C, D), axis=0)
        return x + upd.reshape(B, S, D)

    x = A_x
    x = x + _A_ref(_layernorm(x, axis=-1), A_k_cache, A_v_cache, A_wq, A_wo)
    x = x + _B_ref(_layernorm(x, axis=-1), B_w_r, B_w_gate, B_w_up, B_w_down)
    x = x + _A_ref(_layernorm(x, axis=-1), A_k_cache, A_v_cache, A_wq, A_wo)
    x = x + _B_ref(_layernorm(x, axis=-1), B_w_r, B_w_gate, B_w_up, B_w_down)
    return x
```

```python
import jax
import jax.numpy as jnp
import numpy as np
from jax import lax
import jax.experimental.pallas as pl
import jax.experimental.pallas.tpu as pltpu

B, D, H, SK, DH, F = 4, 640, 32, 4096, 192, 1536
W = min(4096, max(256, SK // 4))
HG = 8
NG = H // HG
GR = HG * DH
HD = H * DH
EPS = 1e-5
SCALE = float(DH) ** -0.5
F32 = jnp.float32
BF16 = jnp.bfloat16


def _layernorm(x):
    m = jnp.mean(x, axis=-1, keepdims=True)
    xc = x - m
    v = jnp.mean(xc * xc, axis=-1, keepdims=True)
    return xc * lax.rsqrt(v + EPS)


def _tiled_dot(lhs, w_ref, k0, nk, n0, nn):
    accs = [None] * nn
    for k in range(nk):
        a = lhs[:, k * 128:(k + 1) * 128]
        for j in range(nn):
            r = jnp.dot(a, w_ref[pl.ds(k0 + k * 128, 128), pl.ds(n0 + j * 128, 128)],
                        preferred_element_type=F32)
            accs[j] = r if k == 0 else accs[j] + r
    return accs


def _kernel(x_ref, wr_ref, k_hbm, v_hbm, wq_hbm, wo_hbm, wg_hbm, wu_hbm, wd_hbm,
            o_ref,
            kbuf, vbuf, wq_v, wo_v, wg_v, wu_v, wd_v, xs, qs, ksem, vsem, wsem):
    def k_copy(b, g):
        return pltpu.make_async_copy(
            k_hbm.at[b, pl.ds(g * GR, GR), pl.ds(SK - W, W)],
            kbuf.at[b, pl.ds(g * GR, GR), :], ksem.at[b, g])

    def v_copy(b, g):
        return pltpu.make_async_copy(
            v_hbm.at[b, pl.ds(g * GR, GR), pl.ds(SK - W, W)],
            vbuf.at[b, pl.ds(g * GR, GR), :], vsem.at[b, g])

    w_copies = [pltpu.make_async_copy(s, d, wsem.at[i]) for i, (s, d) in enumerate(
        [(wq_hbm, wq_v), (wo_hbm, wo_v), (wg_hbm, wg_v), (wu_hbm, wu_v), (wd_hbm, wd_v)])]

    def start_kv(i, _):
        k_copy(i // NG, i % NG).start()
        v_copy(i // NG, i % NG).start()
        return 0

    w_copies[0].start()
    lax.fori_loop(0, NG, start_kv, 0)
    for c in w_copies[1:]:
        c.start()
    lax.fori_loop(NG, B * NG, start_kv, 0)

    xs[0:B, :] = x_ref[...].astype(F32)
    wr = wr_ref[...].astype(F32).reshape(1, D)

    row = lax.broadcasted_iota(jnp.int32, (HG, GR), 0)
    col = lax.broadcasted_iota(jnp.int32, (HG, GR), 1)
    diag = (col >= row * DH) & (col < (row + 1) * DH)
    row8 = lax.broadcasted_iota(jnp.int32, (8, D), 0)

    def attn(b, x, first):
        xn = _layernorm(x).astype(BF16)
        for g in range(NG):
            qa = _tiled_dot(xn, wq_v, 0, D // 128, g * GR, GR // 128)
            qs[:, g * GR:(g + 1) * GR] = jnp.concatenate(qa, axis=1)

        def group(g, acc):
            qg = jnp.where(diag, qs[:, pl.ds(pl.multiple_of(g * GR, 128), GR)], 0.0).astype(BF16)

            @pl.when(first)
            def _():
                k_copy(b, g).wait()

            r0 = pl.multiple_of(g * GR, GR)
            s = jnp.concatenate(_tiled_dot(qg, kbuf.at[b], r0, GR // 128, 0, W // 128), axis=1) * SCALE
            m = jnp.max(s, axis=-1, keepdims=True)
            e = jnp.exp(s - m)
            l = jnp.sum(e, axis=-1, keepdims=True)
            p = (e / l).astype(BF16)

            @pl.when(first)
            def _():
                v_copy(b, g).wait()

            o = lax.dot_general(p, vbuf[b, pl.ds(r0, GR), :], (((1,), (1,)), ((), ())),
                                preferred_element_type=F32)
            og = jnp.where(diag, o, 0.0).astype(BF16)

            @pl.when(first & (b == 0) & (g == 0))
            def _():
                w_copies[1].wait()

            return acc + jnp.concatenate(_tiled_dot(og, wo_v, r0, GR // 128, 0, D // 128), axis=1)

        acc = lax.fori_loop(0, NG, group, jnp.zeros((8, D), F32))
        return x + jnp.sum(acc, axis=0, keepdims=True)

    def ffn(x):
        xn = _layernorm(x)
        r = jnp.sum(xn * wr, axis=-1, keepdims=True)
        xb = xn.astype(BF16)
        gt = jnp.concatenate(_tiled_dot(xb, wg_v, 0, D // 128, 0, F // 128), axis=1)
        up = jnp.concatenate(_tiled_dot(xb, wu_v, 0, D // 128, 0, F // 128), axis=1)
        h = (gt * jax.nn.sigmoid(gt) * up).astype(BF16)
        y = jnp.concatenate(_tiled_dot(h, wd_v, 0, F // 128, 0, D // 128), axis=1)
        return x + (xn + y * jax.nn.sigmoid(r))

    def step(it, carry):
        x, out = carry
        b = it // 2
        first = (it % 2) == 0
        xb0 = jnp.broadcast_to(xs[pl.ds(b, 1), :], (8, D))
        x = jnp.where(first, xb0, x)

        @pl.when(it == 0)
        def _():
            w_copies[0].wait()

        x = attn(b, x, first)

        @pl.when(it == 0)
        def _():
            for c in w_copies[2:]:
                c.wait()

        x = ffn(x)
        out = jnp.where(row8 == b, x, out)
        return x, out

    z = jnp.zeros((8, D), F32)
    _, out = lax.fori_loop(0, 2 * B, step, (z, z))
    o_ref[...] = out[0:B, :].astype(BF16)


@jax.jit
def pallas_interleave_layers__sliding_block_cached__moe_arch_mod__decode_kernel(
    A_x, A_k_cache, A_v_cache, A_wq, A_wo, B_x, B_w_r, B_w_gate, B_w_up, B_w_down,
):
    del B_x
    kT = jnp.swapaxes(A_k_cache, 2, 3).reshape(B, HD, SK)
    vT = jnp.swapaxes(A_v_cache, 2, 3).reshape(B, HD, SK)
    x2 = A_x.reshape(B, D)
    any_spec = pl.BlockSpec(memory_space=pl.ANY)
    vmem_spec = pl.BlockSpec(memory_space=pltpu.VMEM)
    out = pl.pallas_call(
        _kernel,
        in_specs=[vmem_spec, vmem_spec] + [any_spec] * 7,
        out_specs=vmem_spec,
        out_shape=jax.ShapeDtypeStruct((B, D), BF16),
        scratch_shapes=[
            pltpu.VMEM((B, HD, W), BF16),
            pltpu.VMEM((B, HD, W), BF16),
            pltpu.VMEM((D, HD), BF16),
            pltpu.VMEM((HD, D), BF16),
            pltpu.VMEM((D, F), BF16),
            pltpu.VMEM((D, F), BF16),
            pltpu.VMEM((F, D), BF16),
            pltpu.VMEM((8, D), F32),
            pltpu.VMEM((8, HD), F32),
            pltpu.SemaphoreType.DMA((B, NG)),
            pltpu.SemaphoreType.DMA((B, NG)),
            pltpu.SemaphoreType.DMA((5,)),
        ],
        compiler_params=pltpu.CompilerParams(vmem_limit_bytes=127 * 1024 * 1024),
    )(x2, B_w_r, kT, vT, A_wq, A_wo, B_w_gate, B_w_up, B_w_down)
    return out.reshape(B, 1, D)
```

```python
import jax
import jax.numpy as jnp
import numpy as np
from jax import lax
import jax.experimental.pallas as pl
import jax.experimental.pallas.tpu as pltpu

B, D, H, SK, DH, F = 4, 640, 32, 4096, 192, 1536
W = min(4096, max(256, SK // 4))
HG = 8
NG = H // HG
GR = HG * DH
PR = 2 * DH
HD = H * DH
EPS = 1e-5
SCALE = float(DH) ** -0.5
F32 = jnp.float32
BF16 = jnp.bfloat16
U32 = jnp.uint32
RED = 'mxu'
G2 = 4
PLAN = '212kqso'


def _layernorm(x):
    m = jnp.mean(x, axis=-1, keepdims=True)
    xc = x - m
    v = jnp.mean(xc * xc, axis=-1, keepdims=True)
    return xc * lax.rsqrt(v + EPS)


def _wtile(w_ref, k, j):
    return w_ref[pl.ds(k * 128, 128), pl.ds(j * 128, 128)]


def _gdot(lhs, w_ref, k0, nk, j0, nj, out):
    accs = [None] * nj
    for k in range(nk):
        a = lhs[:, k * 128:(k + 1) * 128].astype(BF16)
        for j in range(nj):
            r = jnp.dot(a, _wtile(w_ref, k0 + k, j0 + j), preferred_element_type=F32)
            accs[j] = r if k == 0 else accs[j] + r
            yield
    out(jnp.concatenate(accs, axis=1))


def _dot(lhs, w_ref, k0, nk, j0, nj):
    res = []
    for _ in _gdot(lhs, w_ref, k0, nk, j0, nj, res.append):
        pass
    return res[0]


def _seq(*items):
    def gen():
        for it in items:
            yield from it[1]
    return sum(i[0] for i in items), gen()


def _run(*streams):
    prog = [0] * len(streams)
    live = [True] * len(streams)
    while any(live):
        i = min((prog[k] / streams[k][0], k) for k in range(len(streams)) if live[k])[1]
        try:
            next(streams[i][1])
            prog[i] += 1
        except StopIteration:
            live[i] = False


def _kernel(x_hbm, wr_hbm, k_hbm, v_hbm, wq_hbm, wo_hbm, wg_hbm, wu_hbm, wd_hbm,
            o_ref,
            kbuf, vbuf, wq_v, wo_v, wg_v, wu_v, wd_v, x_v, wr_v, xs, ksem, vsem, wsem):
    k32, v32 = k_hbm, v_hbm

    def k_copy(b, g):
        return pltpu.make_async_copy(
            k32.at[b, pl.ds(g * GR, GR), pl.ds(SK - W, W)],
            kbuf.at[b, pl.ds(g * GR, GR), :], ksem.at[b, g])

    def v_copy(b, g):
        return pltpu.make_async_copy(
            v32.at[b, pl.ds(g * GR, GR), pl.ds(SK - W, W)],
            vbuf.at[b, pl.ds(g * GR, GR), :], vsem.at[b, g])

    def vp_copy(b, p):
        r0 = (NG - 1) * GR + p * PR
        return pltpu.make_async_copy(
            v32.at[b, pl.ds(r0, PR), pl.ds(SK - W, W)],
            vbuf.at[b, pl.ds(r0, PR), :], vsem.at[b, NG - 1 + p])

    w_copies = [pltpu.make_async_copy(s, d, wsem.at[i]) for i, (s, d) in enumerate(
        [(wq_hbm, wq_v), (wo_hbm, wo_v), (wg_hbm, wg_v), (wu_hbm, wu_v), (wd_hbm, wd_v)])]
    x_copy = pltpu.make_async_copy(x_hbm, x_v, wsem.at[5])
    wr_copy = pltpu.make_async_copy(wr_hbm, wr_v, wsem.at[6])

    NCH = 2 * (NG - 1) + 1 + GR // PR

    def start_kv(i, _):
        b, c = i // NCH, i % NCH
        is_k = (c <= 2 * (NG - 1)) & (c % 2 == 0)
        is_v = (c < 2 * (NG - 1)) & (c % 2 == 1)

        @pl.when(is_k)
        def _():
            k_copy(b, c // 2).start()

        @pl.when(is_v)
        def _():
            v_copy(b, c // 2).start()

        @pl.when(c > 2 * (NG - 1))
        def _():
            vp_copy(b, c - 2 * (NG - 1) - 1).start()
        return 0

    w_copies[0].start()

    def start_small(i, _):
        x_copy.start()
        wr_copy.start()
        return 0
    lax.fori_loop(0, 1, start_small, 0)
    lax.fori_loop(0, NCH, start_kv, 0)
    for c in w_copies[1:]:
        c.start()
    lax.fori_loop(NCH, B * NCH, start_kv, 0)

    x_copy.wait()
    wr_copy.wait()
    xs[0:B, :] = x_v[...].astype(F32)
    wr = wr_v[...].astype(F32).reshape(1, D)

    row = lax.broadcasted_iota(jnp.int32, (HG, GR), 0)
    col = lax.broadcasted_iota(jnp.int32, (HG, GR), 1)
    diag = (col >= row * DH) & (col < (row + 1) * DH)
    row8 = lax.broadcasted_iota(jnp.int32, (8, D), 0)
    ones = jnp.ones((8, 128), BF16)

    def softmax(s):
        m = jnp.max(s, axis=-1, keepdims=True)
        e = jnp.exp(s - m)
        l = jnp.sum(e, axis=-1, keepdims=True)
        return e, l

    def ln_stats(x):
        m = jnp.mean(x, axis=-1, keepdims=True)
        xc = x - m
        v = jnp.mean(xc * xc, axis=-1, keepdims=True)
        return m, lax.rsqrt(v + EPS)

    def with_ones(x):
        return jnp.where(row8 == 7, 1.0, x)

    def ln_fix(y, m, rstd):
        cs = jnp.broadcast_to(y[7:8, :], y.shape)
        return (y - m * cs) * rstd

    def attn1(b, x):
        xn = _layernorm(x)
        acc = jnp.zeros((8, D), F32)
        for g in range(NG):
            q = _dot(xn, wq_v, 0, D // 128, g * (GR // 128), GR // 128)
            qg = jnp.where(diag, q, 0.0)
            k_copy(b, g).wait()
            s = _dot(qg, kbuf.at[b], g * (GR // 128), GR // 128, 0, W // 128) * SCALE
            e, l = softmax(s)
            p = e.astype(BF16)
            inv = 1.0 / l
            if g == 0:
                @pl.when(b == 0)
                def _():
                    w_copies[1].wait()
            for pr in range(GR // PR):
                if g < NG - 1:
                    if pr == 0:
                        v_copy(b, g).wait()
                else:
                    vp_copy(b, pr).wait()
                r0 = g * GR + pr * PR
                vt = vbuf[b, pl.ds(r0, PR), :]
                o = lax.dot_general(p, vt, (((1,), (1,)), ((), ())), preferred_element_type=F32)
                og = jnp.where(diag[:, pr * PR:(pr + 1) * PR], o * inv, 0.0)
                acc = acc + _dot(og, wo_v, r0 // 128, PR // 128, 0, D // 128)
        return x + jnp.sum(acc, axis=0, keepdims=True)

    def attn2(b, x):
        xo = with_ones(x)
        m2, rstd2 = ln_stats(x)
        st = {}
        R = G2 * DH
        KT = R // 128
        NU = H // G2
        dg = diag[:, :R]

        def wq(u):
            def fin(q):
                qq = jnp.broadcast_to(q[0:1, :], q.shape) - m2 * jnp.broadcast_to(q[7:8, :], q.shape)
                st['q', u] = jnp.where(dg, qq, 0.0)
            return 5 * KT, _gdot(xo, wq_v, 0, D // 128, u * KT, KT, fin)

        def qk(u):
            def gen():
                def fin(s):
                    st['s', u] = s * (SCALE * rstd2)
                yield from _gdot(st['q', u], kbuf.at[b], u * KT, KT, 0, W // 128, fin)
            return 8 * KT, gen()

        def sm(u):
            def gen():
                e, l = softmax(st['s', u])
                st['e', u] = e
                st['inv', u] = jnp.sum(jnp.where(dg, 1.0 / l, 0.0), axis=0, keepdims=True)
                yield
            return 1, gen()

        def wo(u):
            def gen():
                def fin(y):
                    st['acc'] = y if u == 0 else st['acc'] + y
                yield from _gdot(st['o', u], wo_v, u * KT, KT, 0, D // 128, fin)
            return 5 * KT, gen()

        def pv(u):
            def gen():
                e = st['e', u]
                outs, rows = [], []
                for h in range(G2):
                    pb = [jnp.broadcast_to(e[h:h + 1, j * 256:(j + 1) * 256], (8, 256)) for j in range(W // 256)]
                    for r in range(DH // 16):
                        pair = []
                        for half in range(2):
                            r0 = u * R + h * DH + r * 16 + half * 8
                            acc = None
                            for j in range(W // 256):
                                t = vbuf[b, pl.ds(r0, 8), pl.ds(j * 256, 256)].astype(F32) * pb[j]
                                acc = t if j == 0 else acc + t
                            pair.append(acc[:, :128] + acc[:, 128:])
                        acc = jnp.concatenate(pair, axis=0)
                        rows.append(acc.astype(BF16) if RED == 'mxu' else acc)
                        if len(rows) == 8:
                            blk = jnp.concatenate(rows, axis=0)
                            if RED == 'mxu':
                                outs.append(lax.dot_general(ones, blk, (((1,), (1,)), ((), ())),
                                                            preferred_element_type=F32))
                            else:
                                t = blk.T
                                outs.append(sum(t[8 * i:8 * i + 8] for i in range(1, 16)) + t[0:8])
                            rows = []
                        yield
                st['o', u] = jnp.concatenate(outs, axis=1) * st['inv', u]
            return 12 * G2, gen()

        def ok(f, u):
            return [f(u)] if 0 <= u < NU else []

        lq, lp, lo = (int(c) for c in PLAN[:3])
        order = PLAN[3:]
        for u in range(lq):
            _run(wq(u))
        for t in range(NU + lo):
            items = {'k': ok(qk, t), 'q': ok(wq, t + lq), 'o': ok(wo, t - lo), 's': ok(sm, t)}
            mx = [i for c in order for i in items[c]]
            vp = ok(pv, t - lp)
            streams = ([_seq(*mx)] if mx else []) + vp
            _run(*streams)
        if RED == 'mxu':
            return x + st['acc']
        return x + jnp.sum(st['acc'], axis=0, keepdims=True)

    def ffn(x):
        xo = with_ones(x)
        m, rstd = ln_stats(x)
        xn = (x - m) * rstd
        r = jnp.sum(xn * wr, axis=-1, keepdims=True)
        nh = F // 256
        hs = []
        for c in range(2):
            gt = ln_fix(_dot(xo, wg_v, 0, D // 128, c * nh, nh), m, rstd)
            up = ln_fix(_dot(xo, wu_v, 0, D // 128, c * nh, nh), m, rstd)
            hs.append(gt * jax.nn.sigmoid(gt) * up)
        h = jnp.concatenate(hs, axis=1)
        y = _dot(h, wd_v, 0, F // 128, 0, D // 128)
        out = x + (xn + y * jax.nn.sigmoid(r))
        return jnp.broadcast_to(out[0:1, :], out.shape)

    w_copies[0].wait()

    def step(b, out):
        x = jnp.broadcast_to(xs[pl.ds(b, 1), :], (8, D))
        x = attn1(b, x)

        @pl.when(b == 0)
        def _():
            for c in w_copies[2:]:
                c.wait()

        x = ffn(x)
        x = attn2(b, x)
        x = ffn(x)
        return jnp.where(row8 == b, x, out)

    out = lax.fori_loop(0, B, step, jnp.zeros((8, D), F32))
    o_ref[...] = out[0:B, :].astype(BF16)


@jax.jit
def pallas_interleave_layers__sliding_block_cached__moe_arch_mod__decode_kernel(
    A_x, A_k_cache, A_v_cache, A_wq, A_wo, B_x, B_w_r, B_w_gate, B_w_up, B_w_down,
):
    del B_x
    kT = jnp.swapaxes(A_k_cache, 2, 3).reshape(B, HD, SK)
    vT = jnp.swapaxes(A_v_cache, 2, 3).reshape(B, HD, SK)
    x2 = A_x.reshape(B, D)
    any_spec = pl.BlockSpec(memory_space=pl.ANY)
    vmem_spec = pl.BlockSpec(memory_space=pltpu.VMEM)
    out = pl.pallas_call(
        _kernel,
        in_specs=[any_spec] * 9,
        out_specs=vmem_spec,
        out_shape=jax.ShapeDtypeStruct((B, D), BF16),
        scratch_shapes=[
            pltpu.VMEM((B, HD, W), BF16),
            pltpu.VMEM((B, HD, W), BF16),
            pltpu.VMEM((D, HD), BF16),
            pltpu.VMEM((HD, D), BF16),
            pltpu.VMEM((D, F), BF16),
            pltpu.VMEM((D, F), BF16),
            pltpu.VMEM((F, D), BF16),
            pltpu.VMEM((B, D), BF16),
            pltpu.VMEM((D,), BF16),
            pltpu.VMEM((8, D), F32),
            pltpu.SemaphoreType.DMA((B, NG)),
            pltpu.SemaphoreType.DMA((B, NG - 1 + GR // PR)),
            pltpu.SemaphoreType.DMA((7,)),
        ],
        compiler_params=pltpu.CompilerParams(vmem_limit_bytes=127 * 1024 * 1024, disable_bounds_checks=True, disable_semaphore_checks=True),
    )(x2, B_w_r, kT, vT, A_wq, A_wo, B_w_gate, B_w_up, B_w_down)
    return out.reshape(B, 1, D)
```

```python
import jax
import jax.numpy as jnp
from jax import lax
import jax.experimental.pallas as pl
import jax.experimental.pallas.tpu as pltpu

B, D, H, SK, DH, F = 4, 640, 32, 4096, 192, 1536
W = min(4096, max(256, SK // 4))
HG = 8
NG = H // HG
GR = HG * DH
PR = 2 * DH
HD = H * DH
EPS = 1e-5
SCALE = float(DH) ** -0.5
F32 = jnp.float32
BF16 = jnp.bfloat16
U32 = jnp.uint32

RED = 'xlu'
G2 = 2
PLAN = '225kqso'
WA = 640


def _tile_bf16(w_ref, k, j):
    return w_ref[pl.ds(k * 128, 128), pl.ds(j * 128, 128)]


def _tile_packed(w_ref, k, j):
    return pltpu.bitcast(w_ref[pl.ds(k * 64, 64), pl.ds(j * 128, 128)], BF16)


def _gdot(lhs, tile, nk, nj, out):
    accs = [None] * nj
    for k in range(nk):
        a = lhs[:, k * 128:(k + 1) * 128].astype(BF16)
        for j in range(nj):
            r = jnp.dot(a, tile(k, j), preferred_element_type=F32)
            accs[j] = r if k == 0 else accs[j] + r
            yield
    out(jnp.concatenate(accs, axis=1))


def _dot(lhs, tile, nk, nj):
    res = []
    for _ in _gdot(lhs, tile, nk, nj, res.append):
        pass
    return res[0]


def _seq(*items):
    def gen():
        for it in items:
            yield from it[1]
    return sum(i[0] for i in items), gen()


def _run(*streams):
    prog = [0] * len(streams)
    live = [True] * len(streams)
    while any(live):
        i = min((prog[k] / streams[k][0], k) for k in range(len(streams)) if live[k])[1]
        try:
            next(streams[i][1])
            prog[i] += 1
        except StopIteration:
            live[i] = False


def _kernel(x_hbm, wr_hbm, k_hbm, v_hbm, wq_hbm, wo_hbm, wg_hbm, wu_hbm, wd_hbm,
            o_ref,
            kbuf, vbuf, krep, wq_v, wo_v, wq_p, wo_p, wg_v, wu_v, wd_v, x_v, wr_v, xs,
            ksem, vsem, wsem):
    NP = GR // PR
    LV = (NG - 1) * GR

    def k_copy(b, g):
        return pltpu.make_async_copy(
            k_hbm.at[b, pl.ds(g * GR, GR), pl.ds(SK - W, W)],
            kbuf.at[b % 2, pl.ds(g * GR, GR), :], ksem.at[b, g])

    def v_copy(b, g):
        return pltpu.make_async_copy(
            v_hbm.at[b, pl.ds(g * GR, GR), pl.ds(SK - W, W)],
            vbuf.at[b % 2, pl.ds(g * GR, GR), :], vsem.at[b, g])

    def vp_copy(b, p):
        r0 = LV + p * PR
        return pltpu.make_async_copy(
            v_hbm.at[b, pl.ds(r0, PR), pl.ds(SK - W, W)],
            vbuf.at[b % 2, pl.ds(r0, PR), :], vsem.at[b, NG - 1 + p])

    def vl_copy(b, c0, nc, s):
        r0 = LV + (NP - 1) * PR
        return pltpu.make_async_copy(
            v_hbm.at[b, pl.ds(r0, PR), pl.ds(SK - W + c0, nc)],
            vbuf.at[b % 2, pl.ds(r0, PR), pl.ds(c0, nc)], vsem.at[b, NG - 1 + NP - 1 + s])

    w_copies = [pltpu.make_async_copy(s, d, wsem.at[i]) for i, (s, d) in enumerate(
        [(wq_hbm, wq_v), (wo_hbm, wo_v), (wg_hbm, wg_v), (wu_hbm, wu_v), (wd_hbm, wd_v)])]
    x_copy = pltpu.make_async_copy(x_hbm, x_v, wsem.at[5])
    wr_copy = pltpu.make_async_copy(wr_hbm, wr_v, wsem.at[6])

    NCH = 2 * (NG - 1) + 1 + NP + 1

    def start_kv(i, _):
        b, c = i // NCH, i % NCH
        nkv = 2 * (NG - 1)

        @pl.when((c <= nkv) & (c % 2 == 0))
        def _():
            k_copy(b, c // 2).start()

        @pl.when((c < nkv) & (c % 2 == 1))
        def _():
            v_copy(b, c // 2).start()

        @pl.when((c > nkv) & (c < nkv + NP))
        def _():
            vp_copy(b, c - nkv - 1).start()

        @pl.when(c == nkv + NP)
        def _():
            vl_copy(b, 0, WA, 0).start()

        @pl.when(c == nkv + NP + 1)
        def _():
            vl_copy(b, WA, W - WA, 1).start()
        return 0

    w_copies[0].start()

    def start_small(i, _):
        x_copy.start()
        wr_copy.start()
        return 0
    lax.fori_loop(0, 1, start_small, 0)
    lax.fori_loop(0, NCH, start_kv, 0)
    for c in w_copies[1:]:
        c.start()
    lax.fori_loop(NCH, 2 * NCH, start_kv, 0)

    x_copy.wait()
    wr_copy.wait()
    xs[0:B, :] = x_v[...].astype(F32)
    wr = wr_v[...].astype(F32).reshape(1, D)

    row = lax.broadcasted_iota(jnp.int32, (HG, GR), 0)
    col = lax.broadcasted_iota(jnp.int32, (HG, GR), 1)
    diag = (col >= row * DH) & (col < (row + 1) * DH)
    row8 = lax.broadcasted_iota(jnp.int32, (8, D), 0)
    ones = jnp.ones((8, 128), BF16)

    def repack(src, dst, nk, nj):
        def body(k, _):
            r = pl.multiple_of(k * 128, 128)
            rp = pl.multiple_of(k * 64, 64)
            for j in range(nj):
                t = src[pl.ds(r, 128), pl.ds(j * 128, 128)]
                dst[pl.ds(rp, 64), pl.ds(j * 128, 128)] = pltpu.bitcast(t, U32)
            return 0
        lax.fori_loop(0, nk, body, 0)

    def softmax(s):
        m = jnp.max(s, axis=-1, keepdims=True)
        e = jnp.exp(s - m)
        l = jnp.sum(e, axis=-1, keepdims=True)
        return e, l

    def ln_stats(x):
        m = jnp.mean(x, axis=-1, keepdims=True)
        xc = x - m
        v = jnp.mean(xc * xc, axis=-1, keepdims=True)
        return m, lax.rsqrt(v + EPS)

    def with_ones(x):
        return jnp.where(row8 == 7, 1.0, x)

    def center(y, m):
        return jnp.broadcast_to(y[0:1, :], y.shape) - m * jnp.broadcast_to(y[7:8, :], y.shape)

    def attn1(b, x):
        sl = b % 2
        xo = with_ones(x)
        m, rstd = ln_stats(x)
        acc = jnp.zeros((8, D), F32)
        for g in range(NG):
            kt0 = g * (GR // 128)
            q = _dot(xo, lambda k, j: _tile_packed(wq_p, k, kt0 + j), D // 128, GR // 128)
            qg = jnp.where(diag, center(q, m), 0.0)
            k_copy(b, g).wait()

            def ktile(k, j):
                t = _tile_bf16(kbuf.at[sl], kt0 + k, j)
                krep[pl.ds((kt0 + k) * 64, 64), pl.ds(j * 128, 128)] = pltpu.bitcast(t, U32)
                return t

            s = _dot(qg, ktile, GR // 128, W // 128) * (SCALE * rstd)
            e, l = softmax(s)
            p = e.astype(BF16)
            inv = 1.0 / l
            if g == 0:
                @pl.when(b == 0)
                def _():
                    w_copies[1].wait()
                    repack(wo_v, wo_p, HD // 128, D // 128)
            for pr in range(NP):
                r0 = g * GR + pr * PR
                nt = (((1,), (1,)), ((), ()))
                if g < NG - 1:
                    if pr == 0:
                        v_copy(b, g).wait()
                    o = lax.dot_general(p, vbuf[sl, pl.ds(r0, PR), :], nt, preferred_element_type=F32)
                elif pr < NP - 1:
                    vp_copy(b, pr).wait()
                    o = lax.dot_general(p, vbuf[sl, pl.ds(r0, PR), :], nt, preferred_element_type=F32)
                else:
                    vl_copy(b, 0, WA, 0).wait()
                    oa = lax.dot_general(p[:, :WA], vbuf[sl, pl.ds(r0, PR), pl.ds(0, WA)], nt,
                                         preferred_element_type=F32)
                    oa = jnp.where(diag[:, pr * PR:(pr + 1) * PR], oa, 0.0)
                    vl_copy(b, WA, W - WA, 1).wait()
                    o = lax.dot_general(p[:, WA:], vbuf[sl, pl.ds(r0, PR), pl.ds(WA, W - WA)], nt,
                                        preferred_element_type=F32)
                    o = o + oa
                og = jnp.where(diag[:, pr * PR:(pr + 1) * PR], o * inv, 0.0)
                acc = acc + _dot(og, lambda k, j: _tile_packed(wo_p, r0 // 128 + k, j), PR // 128, D // 128)
        return x + jnp.sum(acc, axis=0, keepdims=True)

    def attn2(b, x):
        sl = b % 2
        xo = with_ones(x)
        m2, rstd2 = ln_stats(x)
        st = {}
        R = G2 * DH
        KT = R // 128
        NU = H // G2
        dg = diag[:, :R]

        def wq(u):
            def fin(q):
                st['q', u] = jnp.where(dg, center(q, m2), 0.0)
            return 5 * KT, _gdot(xo, lambda k, j: _tile_packed(wq_p, k, u * KT + j), D // 128, KT, fin)

        def qk(u):
            def gen():
                def fin(s):
                    st['s', u] = s * (SCALE * rstd2)
                yield from _gdot(st['q', u], lambda k, j: _tile_packed(krep, u * KT + k, j), KT, W // 128, fin)
            return 8 * KT, gen()

        def sm(u):
            def gen():
                e, l = softmax(st['s', u])
                st['e', u] = e
                st['inv', u] = jnp.sum(jnp.where(dg, 1.0 / l, 0.0), axis=0, keepdims=True)
                yield
            return 1, gen()

        def wo(u):
            def gen():
                def fin(y):
                    st['acc'] = y if u == 0 else st['acc'] + y
                yield from _gdot(st['o', u], lambda k, j: _tile_packed(wo_p, u * KT + k, j), KT, D // 128, fin)
            return 5 * KT, gen()

        def pv(u):
            def gen():
                e = st['e', u]
                outs, rows = [], []
                for h in range(G2):
                    pb = [jnp.broadcast_to(e[h:h + 1, j * 256:(j + 1) * 256], (8, 256)) for j in range(W // 256)]
                    for r in range(DH // 16):
                        pair = []
                        for half in range(2):
                            r0 = u * R + h * DH + r * 16 + half * 8
                            acc = None
                            for j in range(W // 256):
                                t = vbuf[sl, pl.ds(r0, 8), pl.ds(j * 256, 256)].astype(F32) * pb[j]
                                acc = t if j == 0 else acc + t
                            pair.append(acc[:, :128] + acc[:, 128:])
                        acc = jnp.concatenate(pair, axis=0)
                        rows.append(acc.astype(BF16) if RED == 'mxu' else acc)
                        if len(rows) == 8:
                            blk = jnp.concatenate(rows, axis=0)
                            if RED == 'mxu':
                                outs.append(lax.dot_general(ones, blk, (((1,), (1,)), ((), ())),
                                                            preferred_element_type=F32))
                            else:
                                t = blk.T
                                outs.append(sum(t[8 * i:8 * i + 8] for i in range(1, 16)) + t[0:8])
                            rows = []
                        yield
                st['o', u] = jnp.concatenate(outs, axis=1) * st['inv', u]
            return 12 * G2, gen()

        def ok(f, u):
            return [f(u)] if 0 <= u < NU else []

        lq, lp, lo = (int(c) for c in PLAN[:3])
        for u in range(lq):
            _run(wq(u))
        for t in range(NU + lo):
            items = {'k': ok(qk, t), 'q': ok(wq, t + lq), 'o': ok(wo, t - lo), 's': ok(sm, t)}
            mx = [i for c in PLAN[3:] for i in items[c]]
            _run(*(([_seq(*mx)] if mx else []) + ok(pv, t - lp)))
        if RED == 'mxu':
            return x + st['acc']
        return x + jnp.sum(st['acc'], axis=0, keepdims=True)

    def ffn(x):
        xo = with_ones(x)
        m, rstd = ln_stats(x)
        xn = (x - m) * rstd
        r = jnp.sum(xn * wr, axis=-1, keepdims=True)
        nh = F // 256
        hs = []
        for c in range(2):
            gt = _dot(xo, lambda k, j: _tile_bf16(wg_v, k, c * nh + j), D // 128, nh)
            up = _dot(xo, lambda k, j: _tile_bf16(wu_v, k, c * nh + j), D // 128, nh)
            gt = (gt - m * jnp.broadcast_to(gt[7:8, :], gt.shape)) * rstd
            up = (up - m * jnp.broadcast_to(up[7:8, :], up.shape)) * rstd
            hs.append(gt * jax.nn.sigmoid(gt) * up)
        h = jnp.concatenate(hs, axis=1)
        y = _dot(h, lambda k, j: _tile_bf16(wd_v, k, j), F // 128, D // 128)
        out = x + (xn + y * jax.nn.sigmoid(r))
        return jnp.broadcast_to(out[0:1, :], out.shape)

    w_copies[0].wait()
    repack(wq_v, wq_p, D // 128, HD // 128)

    def step(b, out):
        x = jnp.broadcast_to(xs[pl.ds(b, 1), :], (8, D))
        x = attn1(b, x)

        @pl.when(b == 0)
        def _():
            for c in w_copies[2:]:
                c.wait()

        x = ffn(x)
        x = attn2(b, x)
        x = ffn(x)

        @pl.when(b + 2 < B)
        def _():
            lax.fori_loop((b + 2) * NCH, (b + 3) * NCH, start_kv, 0)

        return jnp.where(row8 == b, x, out)

    out = lax.fori_loop(0, B, step, jnp.zeros((8, D), F32))
    o_ref[...] = out[0:B, :].astype(BF16)


@jax.jit
def pallas_interleave_layers__sliding_block_cached__moe_arch_mod__decode_kernel(
    A_x, A_k_cache, A_v_cache, A_wq, A_wo, B_x, B_w_r, B_w_gate, B_w_up, B_w_down,
):
    del B_x
    kT = jnp.swapaxes(A_k_cache, 2, 3).reshape(B, HD, SK)
    vT = jnp.swapaxes(A_v_cache, 2, 3).reshape(B, HD, SK)
    x2 = A_x.reshape(B, D)
    any_spec = pl.BlockSpec(memory_space=pl.ANY)
    vmem_spec = pl.BlockSpec(memory_space=pltpu.VMEM)
    out = pl.pallas_call(
        _kernel,
        in_specs=[any_spec] * 9,
        out_specs=vmem_spec,
        out_shape=jax.ShapeDtypeStruct((B, D), BF16),
        scratch_shapes=[
            pltpu.VMEM((2, HD, W), BF16),
            pltpu.VMEM((2, HD, W), BF16),
            pltpu.VMEM((HD // 2, W), U32),
            pltpu.VMEM((D, HD), BF16),
            pltpu.VMEM((HD, D), BF16),
            pltpu.VMEM((D // 2, HD), U32),
            pltpu.VMEM((HD // 2, D), U32),
            pltpu.VMEM((D, F), BF16),
            pltpu.VMEM((D, F), BF16),
            pltpu.VMEM((F, D), BF16),
            pltpu.VMEM((B, D), BF16),
            pltpu.VMEM((D,), BF16),
            pltpu.VMEM((8, D), F32),
            pltpu.SemaphoreType.DMA((B, NG)),
            pltpu.SemaphoreType.DMA((B, NG - 1 + GR // PR + 1)),
            pltpu.SemaphoreType.DMA((7,)),
        ],
        compiler_params=pltpu.CompilerParams(
            vmem_limit_bytes=120 * 1024 * 1024,
            disable_bounds_checks=True, disable_semaphore_checks=True),
    )(x2, B_w_r, kT, vT, A_wq, A_wo, B_w_gate, B_w_up, B_w_down)
    return out.reshape(B, 1, D)
```

```python
import jax
import jax.numpy as jnp
from jax import lax
import jax.experimental.pallas as pl
import jax.experimental.pallas.tpu as pltpu

B, D, H, SK, DH, F = 4, 640, 32, 4096, 192, 1536
W = min(4096, max(256, SK // 4))
HG = 8
NG = H // HG
GR = HG * DH
PR = 2 * DH
HD = H * DH
EPS = 1e-5
SCALE = float(DH) ** -0.5
F32, BF16, U32 = jnp.float32, jnp.bfloat16, jnp.uint32

WA = 640
NV = 4
NQ, UQ = 2, 3
LQ, LP, LO = 2, 2, 5


def _tile(ref, k, j):
    return ref[pl.ds(k * 128, 128), pl.ds(j * 128, 128)]


def _tile_p(ref, k, j):
    return pltpu.bitcast(ref[pl.ds(k * 64, 64), pl.ds(j * 128, 128)], BF16)


def _gdot(lhs, tile, nk, nj, out):
    accs = [None] * nj
    for k in range(nk):
        a = lhs[:, k * 128:(k + 1) * 128].astype(BF16)
        for j in range(nj):
            r = jnp.dot(a, tile(k, j), preferred_element_type=F32)
            accs[j] = r if k == 0 else accs[j] + r
            yield
    out(jnp.concatenate(accs, axis=1))


def _dot(lhs, tile, nk, nj):
    res = []
    for _ in _gdot(lhs, tile, nk, nj, res.append):
        pass
    return res[0]


def _seq(*items):
    def gen():
        for it in items:
            yield from it[1]
    return sum(i[0] for i in items), gen()


def _run(*streams):
    prog = [0] * len(streams)
    live = [True] * len(streams)
    while any(live):
        i = min((prog[k] / streams[k][0], k) for k in range(len(streams)) if live[k])[1]
        try:
            next(streams[i][1])
            prog[i] += 1
        except StopIteration:
            live[i] = False


def _fold16(t):
    return sum(t[8 * i:8 * i + 8] for i in range(1, 16)) + t[0:8]


def _softmax(s):
    m = jnp.max(s, axis=-1, keepdims=True)
    e = jnp.exp(s - m)
    return e, jnp.sum(e, axis=-1, keepdims=True)


def _ln_stats(x):
    m = jnp.mean(x, axis=-1, keepdims=True)
    xc = x - m
    v = jnp.mean(xc * xc, axis=-1, keepdims=True)
    return m, lax.rsqrt(v + EPS)


def _kernel(x_hbm, wr_hbm, k_hbm, v_hbm, wq_hbm, wo_hbm, wg_hbm, wu_hbm, wd_hbm,
            o_ref,
            kbuf, vbuf, krep,
            wq_v, wo_v, wg_v, wu_v, wd_v,
            wq_p, wo_p, wg_p, wu_p, wd_p, wgu_t, wq_t,
            x_v, wr_v, xs, zero, ksem, vsem, wsem):
    NP = GR // PR
    LV = (NG - 1) * GR

    def k_copy(b, g):
        return pltpu.make_async_copy(
            k_hbm.at[b, pl.ds(g * GR, GR), pl.ds(SK - W, W)],
            kbuf.at[b % 2, pl.ds(g * GR, GR), :], ksem.at[b, g])

    def v_copy(b, g):
        return pltpu.make_async_copy(
            v_hbm.at[b, pl.ds(g * GR, GR), pl.ds(SK - W, W)],
            vbuf.at[b % 2, pl.ds(g * GR, GR), :], vsem.at[b, g])

    def vp_copy(b, p):
        r0 = LV + p * PR
        return pltpu.make_async_copy(
            v_hbm.at[b, pl.ds(r0, PR), pl.ds(SK - W, W)],
            vbuf.at[b % 2, pl.ds(r0, PR), :], vsem.at[b, NG - 1 + p])

    def vl_copy(b, c0, nc, s):
        r0 = LV + (NP - 1) * PR
        return pltpu.make_async_copy(
            v_hbm.at[b, pl.ds(r0, PR), pl.ds(SK - W + c0, nc)],
            vbuf.at[b % 2, pl.ds(r0, PR), pl.ds(c0, nc)], vsem.at[b, NG - 1 + NP - 1 + s])

    w_copies = [pltpu.make_async_copy(s, d, wsem.at[i]) for i, (s, d) in enumerate(
        [(wq_hbm, wq_v), (wo_hbm, wo_v), (wg_hbm, wg_v), (wu_hbm, wu_v), (wd_hbm, wd_v)])]
    x_copy = pltpu.make_async_copy(x_hbm, x_v, wsem.at[5])
    wr_copy = pltpu.make_async_copy(wr_hbm, wr_v, wsem.at[6])

    NCH = 2 * (NG - 1) + 1 + NP + 1

    def start_kv(i, _):
        b, c = i // NCH, i % NCH
        nkv = 2 * (NG - 1)

        @pl.when((c <= nkv) & (c % 2 == 0))
        def _():
            k_copy(b, c // 2).start()

        @pl.when((c < nkv) & (c % 2 == 1))
        def _():
            v_copy(b, c // 2).start()

        @pl.when((c > nkv) & (c < nkv + NP))
        def _():
            vp_copy(b, c - nkv - 1).start()

        @pl.when(c == nkv + NP)
        def _():
            vl_copy(b, 0, WA, 0).start()

        @pl.when(c == nkv + NP + 1)
        def _():
            vl_copy(b, WA, W - WA, 1).start()
        return 0

    def start_small(i, _):
        x_copy.start()
        wr_copy.start()
        return 0

    w_copies[0].start()
    lax.fori_loop(0, 1, start_small, 0)
    lax.fori_loop(0, NCH, start_kv, 0)
    for c in w_copies[1:]:
        c.start()
    lax.fori_loop(NCH, 2 * NCH, start_kv, 0)

    zero[0] = 0
    zero[1] = 0
    x_copy.wait()
    wr_copy.wait()
    xs[0:B, :] = x_v[...].astype(F32)
    wr = wr_v[...].astype(F32).reshape(1, D)

    row = lax.broadcasted_iota(jnp.int32, (HG, GR), 0)
    col = lax.broadcasted_iota(jnp.int32, (HG, GR), 1)
    diag = (col >= row * DH) & (col < (row + 1) * DH)
    row8 = lax.broadcasted_iota(jnp.int32, (8, D), 0)

    def repack(src, dst, nk, nj):
        def body(k, _):
            r = pl.multiple_of(k * 128, 128)
            rp = pl.multiple_of(k * 64, 64)
            for j in range(nj):
                t = src[pl.ds(r, 128), pl.ds(j * 128, 128)]
                dst[pl.ds(rp, 64), pl.ds(j * 128, 128)] = pltpu.bitcast(t, U32)
            return 0
        lax.fori_loop(0, nk, body, 0)

    def transposed(src, j, dst, i):
        for k in range(D // 128):
            t = _tile(src, k, j).T
            dst[pl.ds(i * 64, 64), pl.ds(k * 128, 128)] = pltpu.bitcast(t, U32)

    def with_ones(x):
        return jnp.where(row8 == 7, 1.0, x)

    def center(y, m):
        return jnp.broadcast_to(y[0:1, :], y.shape) - m * jnp.broadcast_to(y[7:8, :], y.shape)

    def vpu_dot(xn, wt, nblk, off, out):
        xb = [jnp.broadcast_to(xn[0:1, k * 128:(k + 1) * 128], (16, 128)) for k in range(D // 128)]
        res = []
        for j in range(nblk):
            rows = []
            for r in range(8):
                acc = None
                for k in range(D // 128):
                    w = pltpu.bitcast(wt[pl.ds(off + j * 64 + 8 * r, 8), pl.ds(k * 128, 128)], BF16)
                    t = w.astype(F32) * xb[k]
                    acc = t if k == 0 else acc + t
                rows.append(acc)
                yield
            tot = _fold16(jnp.concatenate(rows, axis=0).T)
            res.append(jnp.broadcast_to(jnp.sum(tot, axis=0, keepdims=True), (8, 128)))
        out(res)

    def attn1(b, x):
        sl = b % 2
        xo = with_ones(x)
        m, rstd = _ln_stats(x)
        acc = jnp.zeros((8, D), F32)
        nt = (((1,), (1,)), ((), ()))
        for g in range(NG):
            kt0 = g * (GR // 128)
            q = _dot(xo, lambda k, j: _tile_p(wq_p, k, kt0 + j), D // 128, GR // 128)
            qg = jnp.where(diag, center(q, m), 0.0)
            k_copy(b, g).wait()

            def ktile(k, j):
                t = _tile(kbuf.at[sl], kt0 + k, j)
                krep[pl.ds((kt0 + k) * 64, 64), pl.ds(j * 128, 128)] = pltpu.bitcast(t, U32)
                return t

            s = _dot(qg, ktile, GR // 128, W // 128) * (SCALE * rstd)
            e, l = _softmax(s)
            p = e.astype(BF16)
            inv = 1.0 / l
            if g == 0:
                @pl.when(b == 0)
                def _():
                    w_copies[1].wait()
                    repack(wo_v, wo_p, HD // 128, D // 128)
            for pr in range(NP):
                r0 = g * GR + pr * PR
                dg = diag[:, pr * PR:(pr + 1) * PR]
                if g < NG - 1:
                    if pr == 0:
                        v_copy(b, g).wait()
                    o = lax.dot_general(p, vbuf[sl, pl.ds(r0, PR), :], nt, preferred_element_type=F32)
                elif pr < NP - 1:
                    vp_copy(b, pr).wait()
                    o = lax.dot_general(p, vbuf[sl, pl.ds(r0, PR), :], nt, preferred_element_type=F32)
                else:
                    vl_copy(b, 0, WA, 0).wait()
                    oa = lax.dot_general(p[:, :WA], vbuf[sl, pl.ds(r0, PR), pl.ds(0, WA)], nt,
                                         preferred_element_type=F32)
                    oa = jnp.where(dg, oa, 0.0)
                    vl_copy(b, WA, W - WA, 1).wait()
                    o = oa + lax.dot_general(p[:, WA:], vbuf[sl, pl.ds(r0, PR), pl.ds(WA, W - WA)], nt,
                                             preferred_element_type=F32)
                og = jnp.where(dg, o * inv, 0.0)
                acc = acc + _dot(og, lambda k, j: _tile_p(wo_p, r0 // 128 + k, j), PR // 128, D // 128)
        return x + jnp.sum(acc, axis=0, keepdims=True)

    def attn2(b, x):
        sl = b % 2
        xo = with_ones(x)
        m2, rstd2 = _ln_stats(x)
        st = {}
        KT = PR // 128
        NU = H // 2
        dg = diag[:, :PR]

        def wq(u):
            def fin(q):
                st['q', u] = jnp.where(dg, center(q, m2), 0.0)
            return 5 * KT, _gdot(xo, lambda k, j: _tile_p(wq_p, k, u * KT + j), D // 128, KT, fin)

        def qk(u):
            def gen():
                def fin(s):
                    st['s', u] = s * (SCALE * rstd2)
                yield from _gdot(st['q', u], lambda k, j: _tile_p(krep, u * KT + k, j), KT, W // 128, fin)
            return 8 * KT, gen()

        def sm(u):
            def gen():
                e, l = _softmax(st['s', u])
                st['e', u] = e
                st['inv', u] = jnp.sum(jnp.where(dg, 1.0 / l, 0.0), axis=0, keepdims=True)
                yield
            return 1, gen()

        def wo(u):
            def gen():
                def fin(y):
                    st['acc'] = y if u == 0 else st['acc'] + y
                yield from _gdot(st['o', u], lambda k, j: _tile_p(wo_p, u * KT + k, j), KT, D // 128, fin)
            return 5 * KT, gen()

        def pv(u):
            def gen():
                e = st['e', u]
                outs, rows = [], []
                for h in range(2):
                    pb = [jnp.broadcast_to(e[h:h + 1, j * 256:(j + 1) * 256], (8, 256))
                          for j in range(W // 256)]
                    for r in range(DH // 16):
                        pair = []
                        for half in range(2):
                            r0 = u * PR + h * DH + r * 16 + half * 8
                            acc = None
                            for j in range(W // 256):
                                t = vbuf[sl, pl.ds(r0, 8), pl.ds(j * 256, 256)].astype(F32) * pb[j]
                                acc = t if j == 0 else acc + t
                            pair.append(acc[:, :128] + acc[:, 128:])
                        rows.append(jnp.concatenate(pair, axis=0))
                        if len(rows) == 8:
                            outs.append(_fold16(jnp.concatenate(rows, axis=0).T))
                            rows = []
                        yield
                st['o', u] = jnp.concatenate(outs, axis=1) * st['inv', u]
            return 24, gen()

        def finq(res):
            for i in range(NQ):
                st['q', UQ + i] = jnp.where(dg, jnp.concatenate(res[3 * i:3 * i + 3], axis=1), 0.0)

        mxu_q = [u for u in range(NU) if not UQ <= u < UQ + NQ]

        def wqm(i):
            return [wq(mxu_q[i])] if i < len(mxu_q) else []

        def ok(f, u):
            return [f(u)] if 0 <= u < NU else []

        _run(_seq(*[i for u in range(LQ) for i in wqm(u)], qk(0)),
             (24 * NQ, vpu_dot(x - m2, wq_t, 3 * NQ, 0, finq)))
        for t in range(NU + LO):
            mx = (ok(qk, t) if t else []) + wqm(t + LQ) + ok(sm, t) + ok(wo, t - LO)
            _run(*(([_seq(*mx)] if mx else []) + ok(pv, t - LP)))
        return x + jnp.sum(st['acc'], axis=0, keepdims=True)

    def ffn(x, which):
        xo = with_ones(x)
        m, rstd = _ln_stats(x)
        xn = (x - m) * rstd
        r = jnp.sum(xn * wr, axis=-1, keepdims=True)
        nm = F // 128 - NV
        h1 = 5
        st = {}

        def keep(key):
            return lambda v: st.__setitem__(key, v)

        def fix(y):
            return (y - m * jnp.broadcast_to(y[7:8, :], y.shape)) * rstd

        def fin(res):
            st['g2'] = jnp.concatenate(res[:NV], axis=1) * rstd
            st['u2'] = jnp.concatenate(res[NV:], axis=1) * rstd

        mx = _seq(
            (5 * h1, _gdot(xo, lambda k, j: _tile_p(wg_p, k, j), D // 128, h1, keep('g0'))),
            (5 * h1, _gdot(xo, lambda k, j: _tile_p(wu_p, k, j), D // 128, h1, keep('u0'))),
            (5 * (nm - h1), _gdot(xo, lambda k, j: _tile_p(wg_p, k, h1 + j), D // 128, nm - h1, keep('g1'))),
            (5 * (nm - h1), _gdot(xo, lambda k, j: _tile_p(wu_p, k, h1 + j), D // 128, nm - h1, keep('u1'))))
        _run(mx, (16 * NV, vpu_dot(x - m, wgu_t, 2 * NV, pl.multiple_of(zero[which], 8), fin)))
        g0, u0, g1, u1 = fix(st['g0']), fix(st['u0']), fix(st['g1']), fix(st['u1'])
        h = jnp.concatenate([g0 * jax.nn.sigmoid(g0) * u0, g1 * jax.nn.sigmoid(g1) * u1,
                             st['g2'] * jax.nn.sigmoid(st['g2']) * st['u2']], axis=1)
        y = _dot(h, lambda k, j: _tile_p(wd_p, k, j), F // 128, D // 128)
        out = x + (xn + y * jax.nn.sigmoid(r))
        return jnp.broadcast_to(out[0:1, :], out.shape)

    w_copies[0].wait()
    repack(wq_v, wq_p, D // 128, HD // 128)
    for j in range(3 * NQ):
        transposed(wq_v, 3 * UQ + j, wq_t, j)

    def step(b, out):
        x = jnp.broadcast_to(xs[pl.ds(b, 1), :], (8, D))
        x = attn1(b, x)

        @pl.when(b == 0)
        def _():
            for c in w_copies[2:]:
                c.wait()
            repack(wg_v, wg_p, D // 128, F // 128)
            repack(wu_v, wu_p, D // 128, F // 128)
            repack(wd_v, wd_p, F // 128, D // 128)
            for i, w_v in enumerate((wg_v, wu_v)):
                for j in range(NV):
                    transposed(w_v, F // 128 - NV + j, wgu_t, i * NV + j)

        x = ffn(x, 0)
        x = attn2(b, x)
        x = ffn(x, 1)

        @pl.when(b + 2 < B)
        def _():
            lax.fori_loop((b + 2) * NCH, (b + 3) * NCH, start_kv, 0)

        return jnp.where(row8 == b, x, out)

    out = lax.fori_loop(0, B, step, jnp.zeros((8, D), F32))
    o_ref[...] = out[0:B, :].astype(BF16)


@jax.jit
def pallas_interleave_layers__sliding_block_cached__moe_arch_mod__decode_kernel(
    A_x, A_k_cache, A_v_cache, A_wq, A_wo, B_x, B_w_r, B_w_gate, B_w_up, B_w_down,
):
    del B_x
    kT = jnp.swapaxes(A_k_cache, 2, 3).reshape(B, HD, SK)
    vT = jnp.swapaxes(A_v_cache, 2, 3).reshape(B, HD, SK)
    out = pl.pallas_call(
        _kernel,
        in_specs=[pl.BlockSpec(memory_space=pl.ANY)] * 9,
        out_specs=pl.BlockSpec(memory_space=pltpu.VMEM),
        out_shape=jax.ShapeDtypeStruct((B, D), BF16),
        scratch_shapes=[
            pltpu.VMEM((2, HD, W), BF16),
            pltpu.VMEM((2, HD, W), BF16),
            pltpu.VMEM((HD // 2, W), U32),
            pltpu.VMEM((D, HD), BF16),
            pltpu.VMEM((HD, D), BF16),
            pltpu.VMEM((D, F), BF16),
            pltpu.VMEM((D, F), BF16),
            pltpu.VMEM((F, D), BF16),
            pltpu.VMEM((D // 2, HD), U32),
            pltpu.VMEM((HD // 2, D), U32),
            pltpu.VMEM((D // 2, F), U32),
            pltpu.VMEM((D // 2, F), U32),
            pltpu.VMEM((F // 2, D), U32),
            pltpu.VMEM((2 * NV * 64, D), U32),
            pltpu.VMEM((3 * NQ * 64, D), U32),
            pltpu.VMEM((B, D), BF16),
            pltpu.VMEM((D,), BF16),
            pltpu.VMEM((8, D), F32),
            pltpu.SMEM((2,), jnp.int32),
            pltpu.SemaphoreType.DMA((B, NG)),
            pltpu.SemaphoreType.DMA((B, NG + GR // PR)),
            pltpu.SemaphoreType.DMA((7,)),
        ],
        compiler_params=pltpu.CompilerParams(
            vmem_limit_bytes=120 * 1024 * 1024,
            disable_bounds_checks=True, disable_semaphore_checks=True),
    )(A_x.reshape(B, D), B_w_r, kT, vT, A_wq, A_wo, B_w_gate, B_w_up, B_w_down)
    return out.reshape(B, 1, D)
```
